```python
import jax
import jax.numpy as jnp

def _softmax(x, axis=-1):
    return jax.nn.softmax(x, axis=axis)
def _gelu(x):
    return jax.nn.gelu(x, approximate=True)
def _silu(x):
    return jax.nn.silu(x)
def _sigmoid(x):
    return jax.nn.sigmoid(x)
def _layernorm(x, axis=-1, eps=1e-5):
    m = jnp.mean(x, axis=axis, keepdims=True)
    v = jnp.var(x, axis=axis, keepdims=True)
    return (x - m) / jnp.sqrt(v + eps)
def _scatter_add(tgt, idx, src, axis=0):
    return tgt.at[idx].add(src)
def _segment_sum(src, seg, n):
    return jax.ops.segment_sum(src, seg, n)
class _Rng:
    def __init__(self, key):
        self._k = key
    def _next(self):
        self._k, sub = jax.random.split(self._k)
        return sub
    def normal(self, shape):
        return jax.random.normal(self._next(), shape, dtype=jnp.bfloat16)
    def randint(self, lo, hi, shape):
        return jax.random.randint(self._next(), shape, lo, hi, dtype=jnp.int32)
    def uniform(self, shape, lo=0.0, hi=1.0):
        return jax.random.uniform(self._next(), shape, jnp.bfloat16, lo, hi)
    def permutation(self, n):
        return jax.random.permutation(self._next(), n)


kernel_name = 'sequential_preLN__sliding_local_dilated__moe_arch_mod__prompt'

def setup_inputs():
    _rng = _Rng(jax.random.key(int.from_bytes(__import__("os").urandom(4), "little")))
    _w = (lambda a: (lambda t: t.astype(jnp.bfloat16) if jnp.issubdtype(t.dtype, jnp.floating) else t)(jnp.asarray(a)))
    def _A_setup():
        B, S, D = 1, 2048, 640
        return {
            "x": _w((lambda *s: _rng.normal(s) * 0.05)(B, S, D)),
            "wqkv": _w((lambda *s: _rng.normal(s) * 0.05)(D, 3 * D)),
            "wo": _w((lambda *s: _rng.normal(s) * 0.05)(D, D)),
        }
    _A_in = _A_setup()

    def _B_setup():
        B, S, D, F, C = 1, 2048, 640, 1536, 1
        return {
            "x": _w((lambda *s: _rng.normal(s) * 0.05)(B, S, D)),
            "w_r": _w((lambda *s: _rng.normal(s) * 0.05)(D)),
            "w_gate": _w((lambda *s: _rng.normal(s) * 0.05)(D, F)),
            "w_up": _w((lambda *s: _rng.normal(s) * 0.05)(D, F)),
            "w_down": _w((lambda *s: _rng.normal(s) * 0.05)(F, D)),
        }
    _B_in = _B_setup()

    return {
        "A_x": _A_in["x"],
        "A_wqkv": _A_in["wqkv"],
        "A_wo": _A_in["wo"],
        "B_x": _B_in["x"],
        "B_w_r": _B_in["w_r"],
        "B_w_gate": _B_in["w_gate"],
        "B_w_up": _B_in["w_up"],
        "B_w_down": _B_in["w_down"],
    }

def reference(A_x, A_wqkv, A_wo, B_x, B_w_r, B_w_gate, B_w_up, B_w_down):
    def _A_ref(x, wqkv, wo):
        B, S, D = x.shape
        H = 32; Dh = D // H
        W, dil = 8, 2
        qkv = (lambda x, *d: x.transpose(*d))((x @ wqkv).reshape(B, S, 3, H, Dh), 2, 0, 3, 1, 4)
        q, k, v = qkv[0], qkv[1], qkv[2]
        scale = Dh ** -0.5
        pos = jnp.arange(S)
        off = jnp.arange(W) * dil
        idx = pos[:, None] - off[None, :]
        mask = idx >= 0
        idx_c = jnp.where(mask, idx, 0).reshape(-1)
        kg = k[:, :, idx_c, :].reshape(B, H, S, W, Dh)
        vg = v[:, :, idx_c, :].reshape(B, H, S, W, Dh)
        logits = jnp.einsum("bhsd,bhswd->bhsw", q, kg) * scale
        logits = jnp.where(mask[None, None, :, :], logits, -1e9)
        attn = _softmax(logits, axis=-1)
        o = jnp.einsum("bhsw,bhswd->bhsd", attn, vg)
        return (lambda x, *d: x.transpose(*d))(o, 0, 2, 1, 3).reshape(B, S, D) @ wo

    def _B_ref(x, w_r, w_gate, w_up, w_down):
        B, S, D = x.shape
        C = 1
        r = x @ w_r
        idx = jnp.argsort(-r, axis=-1)[:, :C]
        idx_e = jnp.repeat(idx.reshape(B, C, 1), D, axis=2)
        x_sel = jnp.take_along_axis(x, idx_e, axis=1)
        g = _silu(x_sel @ w_gate)
        u = x_sel @ w_up
        y = (g * u) @ w_down
        r_sel = _sigmoid(jnp.take_along_axis(r, idx, axis=1))
        y = y * r_sel.reshape(B, C, 1)
        b_off = (jnp.arange(B) * S).reshape(B, 1)
        flat_idx = (idx + b_off).reshape(B * C)
        zero = (x * 0.0).reshape(B * S, D)
        upd = _scatter_add(zero, flat_idx, y.reshape(B * C, D), axis=0)
        return x + upd.reshape(B, S, D)

    x = A_x
    h = x + _A_ref(_layernorm(x, axis=-1), A_wqkv, A_wo)
    h2 = h + _B_ref(_layernorm(h, axis=-1), B_w_r, B_w_gate, B_w_up, B_w_down)
    return h2
```

```python
import math, contextlib

import jax
import jax.numpy as jnp
from jax import lax
import jax.experimental.pallas as pl
import jax.experimental.pallas.tpu as pltpu

S, D, F = 2048, 640, 1536
H, DH = 32, 20
W, DIL = 8, 2
NT = D // 128
HALO = 16
EPS = 1e-5
QSCALE = (DH ** -0.5) * math.log2(math.e)
f32, bf16, u32, i32 = jnp.float32, jnp.bfloat16, jnp.uint32, jnp.int32


def _pack(v):
    return pltpu.bitcast(v.astype(bf16), u32)


def _unpack(v):
    return pltpu.bitcast(v, bf16)


def _ln(v):
    m = jnp.mean(v, axis=-1, keepdims=True)
    c = v - m
    var = jnp.mean(c * c, axis=-1, keepdims=True)
    return c * lax.rsqrt(var + EPS)


def make_kernel(TM=256, AR=16, LR=32, TIE="alc", ASPAN=(0, 1), LSPAN=(0, 0.67), CSPAN=(0, 1), A7=(0, 2), CS=(0, 1), DL=0, DC=0, CLAST=0, PQ=1, XW=0, SCOPES=0, MM=128, NG=(5,), flags=None):
    NB = S // TM
    NSLOT = 4 * NT

    def kernel(x_hbm, wqkv_hbm, wo_hbm, wr_ref, wg_hbm, wu_hbm, wd_hbm, out_hbm,
               x_v, wqkv_v, wo_v, wg_v, wu_v, wd_v,
               wt_u, wp, wo_u, wop,
               xn, qkv, o_v, h_v, out_v, fix_v,
               sem_x, sem_w, sem_m, sem_o, sem_r):

        xcuts = [0, TM, 2 * TM, 3 * TM, S]
        x_cp = [pltpu.make_async_copy(x_hbm.at[pl.ds(a, b - a), :], x_v.at[pl.ds(a, b - a), :], sem_x.at[k])
                for k, (a, b) in enumerate(zip(xcuts[:-1], xcuts[1:]))]

        def w_copy(p):
            return pltpu.make_async_copy(wqkv_hbm.at[:, pl.ds(p * D, D)],
                                         wqkv_v.at[:, pl.ds(p * D, D)], sem_w.at[p])

        misc = [pltpu.make_async_copy(wo_hbm, wo_v, sem_m.at[0]),
                pltpu.make_async_copy(wg_hbm, wg_v, sem_m.at[1]),
                pltpu.make_async_copy(wu_hbm, wu_v, sem_m.at[2]),
                pltpu.make_async_copy(wd_hbm, wd_v, sem_m.at[3])]

        def out_copy(i):
            return pltpu.make_async_copy(out_v.at[pl.ds(i * TM, TM), :],
                                         out_hbm.at[pl.ds(i * TM, TM), :], sem_o.at[i])

        x_cp[0].start()
        w_copy(0).start()

        never = pl.semaphore_read(sem_r) > 0

        def tied(const, mark):
            v = jnp.full((8, 128), const, f32)
            return v if mark is None else jnp.where(never, mark, v)

        def prep_w(p):
            for kt in range(NT):
                wt = wqkv_v[pl.ds(kt * 128, 128), pl.ds(p * D, D)].T
                wt_u[kt, pl.ds(p * 320, 320), :] = pltpu.bitcast(wt, u32)
            for kt in range(NT):
                for j in range(NT):
                    for a in range(2):
                        wp[pl.ds(p * 320 + j * 64 + a * 32, 32), pl.ds(kt * 128, 128)] = (
                            wt_u[kt, pl.ds(p * 320 + 2 * j + a, 32, stride=10), :])

        def prep_wo():
            for nt in range(NT):
                wo_u[nt] = pltpu.bitcast(wo_v[:, pl.ds(nt * 128, 128)], u32)
            for nt in range(NT):
                for j in range(NT):
                    for a in range(2):
                        wop[pl.ds(j * 64 + a * 32, 32), pl.ds(nt * 128, 128)] = (
                            wo_u[nt, pl.ds(2 * j + a, 32, stride=10), :])

        def tiles(v):
            return [v[:, t * 128:(t + 1) * 128] for t in range(NT)]

        def rowsum(ts, mark=None):
            acc = ts[0]
            if mark is not None:
                z = tied(0.0, mark)
                acc = acc + jnp.concatenate([z] * (acc.shape[0] // 8), axis=0)
            for t in ts[1:]:
                acc = acc + t
            return jnp.sum(acc, axis=-1, keepdims=True)

        def ln1_chunk(r0, mark):
            x = x_v[pl.ds(r0, LR), :].astype(f32)
            m = rowsum(tiles(x), mark) * (1.0 / D)
            c = x - m
            var = rowsum(tiles(c * c)) * (1.0 / D)
            xn[pl.ds(r0 // 2, LR // 2), :] = _pack(c * lax.rsqrt(var + EPS))

        def deadline(lhs, deps):
            if not deps:
                return lhs
            d = deps[0]
            for e in deps[1:]:
                d = d | e
            head = jnp.where(never, d, lhs[0:8, 0:128])
            top = jnp.concatenate([head, lhs[0:8, 128:]], axis=1)
            return jnp.concatenate([top, lhs[8:]], axis=0)

        def q_piece(i, t, deps=()):
            m, t0, nt = t
            r0 = i * TM + m * MM
            lhs = _unpack(deadline(xn[pl.ds(r0 // 2, MM // 2), :], deps))
            res = lax.dot_general(lhs, _unpack(wp[pl.ds(t0 * 64, nt * 64), :]),
                                  (((1,), (1,)), ((), ())), preferred_element_type=f32)
            for u in range(nt):
                qkv[t0 + u, pl.ds(HALO + r0, MM), :] = res[:, u * 128:(u + 1) * 128]
            return res[0:8, 0:128]

        def o_piece(i, t, deps=()):
            m, t0, nt = t
            r0 = i * TM + m * MM
            res = jnp.dot(_unpack(deadline(o_v[pl.ds(r0 // 2, MM // 2), :], deps)),
                          _unpack(wop[:, pl.ds(t0 * 128, nt * 128)]), preferred_element_type=f32)
            h_v[pl.ds(r0, MM), pl.ds(t0 * 128, nt * 128)] = (
                res + x_v[pl.ds(r0, MM), pl.ds(t0 * 128, nt * 128)].astype(f32))
            return res[0:8, 0:128]

        def groups(parts):
            out = []
            for m in range(TM // MM):
                for p in parts:
                    t0 = p * NT
                    for g in NG:
                        out.append((m, t0, g))
                        t0 += g
            return out

        lane = lax.broadcasted_iota(i32, (AR, 128), 1)
        swap = lane ^ 1

        def attn_chunk(r0, mark):
            sc = jnp.concatenate([tied(QSCALE, mark)] * (AR // 8), axis=0)
            q = [qkv[t, pl.ds(HALO + r0, AR), :] * sc for t in range(NT)]
            accs = []
            for w in range(W):
                acc = None
                for t in range(NT):
                    e = q[t] * qkv[NT + t, pl.ds(HALO + r0 - DIL * w, AR), :]
                    acc = e if acc is None else acc + e
                accs.append(acc)
            rolled = [pltpu.roll(a, 64, 1) for a in accs]
            accs = [a + r for a, r in zip(accs, rolled)]
            swapped = [jnp.take_along_axis(a, swap, axis=1) for a in accs]
            logits = []
            for w in range(W):
                acc = accs[w] + swapped[w]
                if r0 < DIL * w:
                    row = r0 + lax.broadcasted_iota(i32, (AR, 128), 0)
                    acc = jnp.where(row >= DIL * w, acc, -1e9)
                logits.append(acc)
            m = logits[0]
            for w in range(1, W):
                m = jnp.maximum(m, logits[w])
            es = [jnp.exp2(l - m) for l in logits]
            ssum = es[0]
            for w in range(1, W):
                ssum = ssum + es[w]
            inv = 1.0 / ssum
            done = None
            for t in range(NT):
                acc = None
                for w in range(W):
                    e = es[w] * qkv[2 * NT + t, pl.ds(HALO + r0 - DIL * w, AR), :]
                    acc = e if acc is None else acc + e
                packed = _pack(acc * inv)
                o_v[pl.ds(r0 // 2, AR // 2), pl.ds(t * 128, 128)] = packed
                for g in range(AR // 16):
                    pg = packed[g * 8:(g + 1) * 8]
                    done = pg if done is None else done | pg
            return done

        best = [jnp.full((8, 128), -jnp.inf, f32), jnp.zeros((8, 128), i32)]
        wr = wr_ref[...].astype(f32).reshape(1, D)

        def ln2_chunk(r0, mark):
            h = h_v[pl.ds(r0, LR), :]
            m = rowsum(tiles(h), mark) * (1.0 / D)
            c = h - m
            var = rowsum(tiles(c * c)) * (1.0 / D)
            cw = rowsum(tiles(c * wr))
            rstd = lax.rsqrt(var + EPS)
            out_v[pl.ds(r0, LR), :] = (h + c * rstd).astype(bf16)
            r = jnp.broadcast_to(cw * rstd, (LR, 128))
            bv, bi = best
            for g in range(LR // 8):
                rg = r[g * 8:(g + 1) * 8]
                upd = rg > bv
                bv = jnp.where(upd, rg, bv)
                bi = jnp.where(upd, r0 + g * 8, bi)
            best[0], best[1] = bv, bi
            return pltpu.bitcast(bv, u32)

        zero_halo = jnp.zeros((HALO, 128), f32)
        for t in range(NT, 3 * NT):
            qkv[t, pl.ds(0, HALO), :] = zero_halo

        sc = (lambda n: jax.named_scope(n)) if SCOPES else (lambda n: contextlib.nullcontext())
        gq, gk, gv = groups((0,)), groups((1,)), groups((2,))
        hq = (len(gq) * PQ) // 2
        with sc("p0"):
            x_cp[0].wait()
            w_copy(1).start()
            x_cp[1].start()
            for r0 in range(0, TM, LR):
                ln1_chunk(r0, None)
        with sc("p1w"):
            w_copy(0).wait()
            w_copy(2).start()
            x_cp[2].start()
            misc[0].start()
        with sc("p1p"):
            prep_w(0)
        with sc("p1m"):
            for t in gq[:hq]:
                q_piece(0, t)
        with sc("p2w"):
            w_copy(1).wait()
            x_cp[3].start()
        with sc("p2"):
            prep_w(1)
            for t in gq[hq:] + gk[:hq]:
                q_piece(0, t)
        with sc("p3w"):
            x_cp[1].wait()
            w_copy(2).wait()
            for c in misc[1:]:
                c.start()
        with sc("p3"):
            prep_w(2)
            for r0 in range(TM, 2 * TM, LR):
                ln1_chunk(r0, None)
            for t in gk[hq:] + gv:
                q_piece(0, t)
        with sc("p4"):
            misc[0].wait()
            x_cp[2].wait()
            prep_wo()

        seq = [("q", 1)]
        for i in range(2, NB):
            seq += [("q", i), ("o", i - 2)]
        seq += [("o", NB - 2), ("o", NB - 1)]
        pieces, start = [], {}
        for kind, i in seq:
            start[(kind, i)] = len(pieces)
            pieces += [(kind, i, t) for t in groups((0, 1, 2) if kind == "q" else (0,))]
        n = len(pieces)
        jobs = [[] for _ in range(n + 1)]

        def spread(fn, blk, rows, base, span, tie):
            nc = TM // rows
            for c in range(nc):
                k = base + span[0] + (c * (span[1] - span[0])) // nc + 1
                jobs[min(k, n)].append((fn, blk * TM + c * rows, tie))

        na = TM // AR
        ASPAN_, LSPAN_, CSPAN_ = [(int(a * len(groups((0, 1, 2)))), int(b * len(groups((0, 1, 2))))) for a, b in (ASPAN, LSPAN, CSPAN)]
        A7_, CS_ = [(int(a * len(groups((0,)))), int(b * len(groups((0,))))) for a, b in (A7, CS)]
        for j in range(NB):
            if j + 1 < NB:
                spread(attn_chunk, j, AR, start[("q", j + 1)], ASPAN_, "a" in TIE)
            else:
                spread(attn_chunk, j, AR, start[("o", j - 2)], A7_, "a" in TIE)
            if 2 <= j:
                spread(ln1_chunk, j, LR, start[("q", j - 1)], LSPAN_, "l" in TIE)
            if j + 3 < NB:
                spread(ln2_chunk, j, LR, start[("q", j + 3)], CSPAN_, "c" in TIE)
            elif j + 1 < NB:
                spread(ln2_chunk, j, LR, start[("o", j + 1)], CS_, "c" in TIE)
            else:
                spread(ln2_chunk, j, LR, n, (0, 0), False)
        last_c = {}
        for k in range(n + 1):
            for fn, r0, _ in jobs[k]:
                if fn is ln2_chunk:
                    last_c[r0 // TM] = k
        mark = None
        due = [[] for _ in range(n + 1 + DL + DC)]
        stack = contextlib.ExitStack()
        for k in range(n + 1):
            if k % 12 == 0:
                stack.close()
                stack.enter_context(sc("s%d" % k))
            for fn, r0, tie in jobs[k]:
                done = fn(r0, mark if tie else None)
                if DL and fn is attn_chunk:
                    due[k + DL].append(done)
                if DC and fn is ln2_chunk and (not CLAST or (r0 + LR) % (TM // CLAST) == 0):
                    due[min(k + DC, n)].append(done)
            if k == start[("q", 2)] - XW:
                x_cp[3].wait()
            for j, kk in last_c.items():
                if kk == k:
                    out_copy(j).start()
            if k < n:
                kind, i, t = pieces[k]
                mark = q_piece(i, t, due[k]) if kind == "q" else o_piece(i, t, due[k])

        stack.close()
        stack.enter_context(sc("tail"))
        bv, bi = best
        gmax = jnp.max(bv, axis=0, keepdims=True)
        cand = jnp.where(bv == gmax, bi + lax.broadcasted_iota(i32, (8, 128), 0), S)
        idx = jnp.min(cand)
        base = pl.multiple_of((idx // 16) * 16, 16)
        h16 = h_v[pl.ds(base, 16), :]
        hn16 = _ln(h16)
        sel = (lax.broadcasted_iota(i32, (16, D), 0) + base) == idx
        xs = jnp.where(sel, hn16, 0.0).astype(bf16)
        for c in misc[1:]:
            c.wait()
        g = jnp.dot(xs, wg_v[...], preferred_element_type=f32)
        u = jnp.dot(xs, wu_v[...], preferred_element_type=f32)
        act = (g * jax.nn.sigmoid(g) * u).astype(bf16)
        y = jnp.dot(act, wd_v[...], preferred_element_type=f32)
        rsel = jnp.sum(hn16 * wr, axis=-1, keepdims=True)
        y = y * jax.nn.sigmoid(rsel)
        fix_v[...] = (h16 + jnp.where(sel, hn16 + y, hn16)).astype(bf16)
        for i in range(NB):
            out_copy(i).wait()
        fix = pltpu.make_async_copy(fix_v, out_hbm.at[pl.ds(base, 16), :], sem_o.at[NB])
        fix.start()
        fix.wait()
        stack.close()

    any_spec = pl.BlockSpec(memory_space=pl.ANY)
    scratch = [
        pltpu.VMEM((S, D), bf16),
        pltpu.VMEM((D, 3 * D), bf16),
        pltpu.VMEM((D, D), bf16),
        pltpu.VMEM((D, F), bf16),
        pltpu.VMEM((D, F), bf16),
        pltpu.VMEM((F, D), bf16),
        pltpu.VMEM((NT, 960, 128), u32),
        pltpu.VMEM((960, D), u32),
        pltpu.VMEM((NT, 320, 128), u32),
        pltpu.VMEM((320, D), u32),
        pltpu.VMEM((S // 2, D), u32),
        pltpu.VMEM((3 * NT, S + HALO, 128), f32),
        pltpu.VMEM((S // 2, D), u32),
        pltpu.VMEM((S, D), f32),
        pltpu.VMEM((S, D), bf16),
        pltpu.VMEM((16, D), bf16),
        pltpu.SemaphoreType.DMA((4,)),
        pltpu.SemaphoreType.DMA((3,)),
        pltpu.SemaphoreType.DMA((4,)),
        pltpu.SemaphoreType.DMA((NB + 1,)),
        pltpu.SemaphoreType.REGULAR,
    ]

    def call(A_x, A_wqkv, A_wo, B_x, B_w_r, B_w_gate, B_w_up, B_w_down):
        out = pl.pallas_call(
            kernel,
            out_shape=jax.ShapeDtypeStruct((S, D), bf16),
            grid=(1,),
            in_specs=[any_spec, any_spec, any_spec,
                      pl.BlockSpec((D,), lambda i: (0,)),
                      any_spec, any_spec, any_spec],
            out_specs=any_spec,
            scratch_shapes=scratch,
            compiler_params=pltpu.CompilerParams(vmem_limit_bytes=100 * 1024 * 1024, flags=flags),
        )(A_x.reshape(S, D), A_wqkv, A_wo, B_w_r, B_w_gate, B_w_up, B_w_down)
        return out.reshape(1, S, D)

    return call


_call = make_kernel(TIE='', MM=128, NG=(2,2,1), DL=8, DC=16, CLAST=1)


@jax.jit
def pallas_sequential_preLN__sliding_local_dilated__moe_arch_mod__prompt_kernel(
    A_x: jax.Array,
    A_wqkv: jax.Array,
    A_wo: jax.Array,
    B_x: jax.Array,
    B_w_r: jax.Array,
    B_w_gate: jax.Array,
    B_w_up: jax.Array,
    B_w_down: jax.Array,
):
    return _call(A_x, A_wqkv, A_wo, B_x, B_w_r, B_w_gate, B_w_up, B_w_down)
```

```python
import math, contextlib

import jax
import jax.numpy as jnp
from jax import lax
import jax.experimental.pallas as pl
import jax.experimental.pallas.tpu as pltpu

S, D, F = 2048, 640, 1536
H, DH = 32, 20
W, DIL = 8, 2
NT = D // 128
HALO = 16
EPS = 1e-5
QSCALE = (DH ** -0.5) * math.log2(math.e)
f32, bf16, u32, i32 = jnp.float32, jnp.bfloat16, jnp.uint32, jnp.int32


def _pack(v):
    return pltpu.bitcast(v.astype(bf16), u32)


def _unpack(v):
    return pltpu.bitcast(v, bf16)


def _ln(v):
    m = jnp.mean(v, axis=-1, keepdims=True)
    c = v - m
    var = jnp.mean(c * c, axis=-1, keepdims=True)
    return c * lax.rsqrt(var + EPS)


def make_kernel(TM=256, AR=16, LR=32, TIE="alc", ASPAN=(0, 1), LSPAN=(0, 0.67), CSPAN=(0, 1), A7=(0, 2), CS=(0, 1), DL=0, DC=0, CLAST=0, PQ=1, P0=0, RL='', CH='', CD=1, W1=-3, W2=-3, X1=0, X2=-4, DX=0, ILV=0, SCOPES=0, MM=128, NG=(5,), flags=None):
    NB = S // TM
    NSLOT = 4 * NT

    def kernel(x_hbm, wqkv_hbm, wo_hbm, wr_hbm, wg_hbm, wu_hbm, wd_hbm, out_hbm,
               wr_ref, x_v, wqkv_v, wo_v, wg_v, wu_v, wd_v,
               wt_u, wp, wo_u, wop,
               xn, qkv, o_v, h_v, out_v, fix_v,
               sem_x, sem_w, sem_m, sem_o, sem_r):

        xcuts = [0, TM, 2 * TM, S]
        x_cp = [pltpu.make_async_copy(x_hbm.at[pl.ds(a, b - a), :], x_v.at[pl.ds(a, b - a), :], sem_x.at[k])
                for k, (a, b) in enumerate(zip(xcuts[:-1], xcuts[1:]))]

        def w0_copy(kt):
            return pltpu.make_async_copy(wqkv_hbm.at[pl.ds(kt * 128, 128), pl.ds(0, D)],
                                         wqkv_v.at[pl.ds(kt * 128, 128), pl.ds(0, D)], sem_w.at[3 + kt])

        def w_copy(p):
            return pltpu.make_async_copy(wqkv_hbm.at[:, pl.ds(p * D, D)],
                                         wqkv_v.at[:, pl.ds(p * D, D)], sem_w.at[p])

        misc = [pltpu.make_async_copy(wo_hbm, wo_v, sem_m.at[0]),
                pltpu.make_async_copy(wg_hbm, wg_v, sem_m.at[1]),
                pltpu.make_async_copy(wu_hbm, wu_v, sem_m.at[2]),
                pltpu.make_async_copy(wd_hbm, wd_v, sem_m.at[3])]

        wr_cp = pltpu.make_async_copy(wr_hbm, wr_ref, sem_x.at[3])

        def out_copy(i):
            return pltpu.make_async_copy(out_v.at[pl.ds(i * TM, TM), :],
                                         out_hbm.at[pl.ds(i * TM, TM), :], sem_o.at[i])

        if P0:
            w_copy(0).start()
            x_cp[0].start()
        else:
            x_cp[0].start()
            w_copy(0).start()

        zero = pl.semaphore_read(sem_r)
        never = zero > 0

        def rows(r0, k):
            return pl.ds(pl.multiple_of(r0 + zero * k, LR), LR)

        def tied(const, mark):
            v = jnp.full((8, 128), const, f32)
            return v if mark is None else jnp.where(never, mark, v)

        def prep_w(p, kts=range(NT)):
            for kt in kts:
                wt = wqkv_v[pl.ds(kt * 128, 128), pl.ds(p * D, D)].T
                wt_u[kt, pl.ds(p * 320, 320), :] = pltpu.bitcast(wt, u32)
            for kt in kts:
                for j in range(NT):
                    for a in range(2):
                        wp[pl.ds(p * 320 + j * 64 + a * 32, 32), pl.ds(kt * 128, 128)] = (
                            wt_u[kt, pl.ds(p * 320 + 2 * j + a, 32, stride=10), :])

        def prep_wo():
            for nt in range(NT):
                wo_u[nt] = pltpu.bitcast(wo_v[:, pl.ds(nt * 128, 128)], u32)
            for nt in range(NT):
                for j in range(NT):
                    for a in range(2):
                        wop[pl.ds(j * 64 + a * 32, 32), pl.ds(nt * 128, 128)] = (
                            wo_u[nt, pl.ds(2 * j + a, 32, stride=10), :])

        def tiles(v):
            return [v[:, t * 128:(t + 1) * 128] for t in range(NT)]

        def rowsum(ts, mark=None):
            acc = ts[0]
            if mark is not None:
                z = tied(0.0, mark)
                acc = acc + jnp.concatenate([z] * (acc.shape[0] // 8), axis=0)
            for t in ts[1:]:
                acc = acc + t
            return jnp.sum(acc, axis=-1, keepdims=True)

        chain = {"a": [], "l": [], "c": []}

        def chained(kind, mark):
            if kind in CH and len(chain[kind]) >= CD:
                return chain[kind][-CD]
            return mark

        def ln1_chunk(r0, mark):
            x = x_v[pl.ds(r0, LR), :].astype(f32)
            m = rowsum(tiles(x), chained("l", mark)) * (1.0 / D)
            c = x - m
            chain["l"].append(c[0:8, 0:128])
            if "l" in RL:
                c = x_v[rows(r0, 1), :].astype(f32) - m
            var = rowsum(tiles(c * c)) * (1.0 / D)
            if "l" in RL:
                c = x_v[rows(r0, 2), :].astype(f32) - m
            packed = _pack(c * lax.rsqrt(var + EPS))
            xn[pl.ds(r0 // 2, LR // 2), :] = packed
            return packed[LR // 2 - 8:, D - 128:]

        def deadline(lhs, deps):
            if not deps:
                return lhs
            d = deps[0]
            for e in deps[1:]:
                d = d | e
            head = jnp.where(never, d, lhs[0:8, 0:128])
            top = jnp.concatenate([head, lhs[0:8, 128:]], axis=1)
            return jnp.concatenate([top, lhs[8:]], axis=0)

        def q_piece(i, t, deps=()):
            m, t0, nt = t
            r0 = i * TM + m * MM
            lhs = _unpack(deadline(xn[pl.ds(r0 // 2, MM // 2), :], deps))
            res = lax.dot_general(lhs, _unpack(wp[pl.ds(t0 * 64, nt * 64), :]),
                                  (((1,), (1,)), ((), ())), preferred_element_type=f32)
            for u in range(nt):
                qkv[t0 + u, pl.ds(HALO + r0, MM), :] = res[:, u * 128:(u + 1) * 128]
            return res[0:8, 0:128]

        def o_piece(i, t, deps=()):
            m, t0, nt = t
            r0 = i * TM + m * MM
            res = jnp.dot(_unpack(deadline(o_v[pl.ds(r0 // 2, MM // 2), :], deps)),
                          _unpack(wop[:, pl.ds(t0 * 128, nt * 128)]), preferred_element_type=f32)
            h_v[pl.ds(r0, MM), pl.ds(t0 * 128, nt * 128)] = (
                res + x_v[pl.ds(r0, MM), pl.ds(t0 * 128, nt * 128)].astype(f32))
            return res[0:8, 0:128]

        def groups(parts):
            out = []
            for m in range(TM // MM):
                for p in parts:
                    t0 = p * NT
                    for g in NG:
                        out.append((m, t0, g))
                        t0 += g
            return out

        lane = lax.broadcasted_iota(i32, (AR, 128), 1)
        swap = lane ^ 1

        def attn_chunk(r0, mark):
            mark = chained("a", mark)
            sc = jnp.concatenate([tied(QSCALE, mark)] * (AR // 8), axis=0)
            q = [qkv[t, pl.ds(HALO + r0, AR), :] * sc for t in range(NT)]
            accs = []
            for w in range(W):
                acc = None
                for t in range(NT):
                    e = q[t] * qkv[NT + t, pl.ds(HALO + r0 - DIL * w, AR), :]
                    acc = e if acc is None else acc + e
                accs.append(acc)
            rolled = [pltpu.roll(a, 64, 1) for a in accs]
            accs = [a + r for a, r in zip(accs, rolled)]
            chain["a"].append(accs[-1][0:8])
            swapped = [jnp.take_along_axis(a, swap, axis=1) for a in accs]
            logits = []
            for w in range(W):
                acc = accs[w] + swapped[w]
                if r0 < DIL * w:
                    row = r0 + lax.broadcasted_iota(i32, (AR, 128), 0)
                    acc = jnp.where(row >= DIL * w, acc, -1e9)
                logits.append(acc)
            m = logits[0]
            for w in range(1, W):
                m = jnp.maximum(m, logits[w])
            es = [jnp.exp2(l - m) for l in logits]
            ssum = es[0]
            for w in range(1, W):
                ssum = ssum + es[w]
            inv = 1.0 / ssum
            done = None
            for t in range(NT):
                acc = None
                for w in range(W):
                    e = es[w] * qkv[2 * NT + t, pl.ds(HALO + r0 - DIL * w, AR), :]
                    acc = e if acc is None else acc + e
                packed = _pack(acc * inv)
                o_v[pl.ds(r0 // 2, AR // 2), pl.ds(t * 128, 128)] = packed
                for g in range(AR // 16):
                    pg = packed[g * 8:(g + 1) * 8]
                    done = pg if done is None else done | pg
            return done

        best = [jnp.full((8, 128), -jnp.inf, f32), jnp.zeros((8, 128), i32)]
        wr_box = []

        def get_wr():
            if not wr_box:
                wr_box.append(wr_ref[...].astype(f32).reshape(1, D))
            return wr_box[0]

        def ln2_chunk(r0, mark):
            h = h_v[pl.ds(r0, LR), :]
            m = rowsum(tiles(h), chained("c", mark)) * (1.0 / D)
            c = h - m
            chain["c"].append(c[0:8, 0:128])
            if "c" in RL:
                c = h_v[rows(r0, 1), :] - m
            var = rowsum(tiles(c * c)) * (1.0 / D)
            cw = rowsum(tiles(c * get_wr()))
            rstd = lax.rsqrt(var + EPS)
            if "c" in RL:
                h = h_v[rows(r0, 2), :]
                c = h - m
            out_v[pl.ds(r0, LR), :] = (h + c * rstd).astype(bf16)
            r = jnp.broadcast_to(cw * rstd, (LR, 128))
            bv, bi = best
            for g in range(LR // 8):
                rg = r[g * 8:(g + 1) * 8]
                upd = rg > bv
                bv = jnp.where(upd, rg, bv)
                bi = jnp.where(upd, r0 + g * 8, bi)
            best[0], best[1] = bv, bi
            return pltpu.bitcast(bv, u32)

        zero_halo = jnp.zeros((HALO, 128), f32)
        for t in range(NT, 3 * NT):
            qkv[t, pl.ds(0, HALO), :] = zero_halo

        sc = (lambda n: jax.named_scope(n)) if SCOPES else (lambda n: contextlib.nullcontext())
        with sc("p0"):
            if P0:
                w_copy(0).wait()
                w_copy(1).start()
                wr_cp.start()
                prep_w(0, range(P0))
                x_cp[0].wait()
                w_copy(2).start()
                x_cp[1].start()
                prep_w(0, range(P0, NT))
                for r0 in range(0, TM, LR):
                    ln1_chunk(r0, None)
            else:
                x_cp[0].wait()
                w_copy(1).start()
                wr_cp.start()
                for r0 in range(0, TM, LR):
                    ln1_chunk(r0, None)
                w_copy(0).wait()
                w_copy(2).start()
                x_cp[1].start()
                prep_w(0)

        nm = TM // MM
        seq = [("q", 0, (p,)) for p in range(3)] + [("q", 1, (0, 1, 2))]
        for i in range(2, NB):
            seq += [("q", i, (0, 1, 2)), ("o", i - 2, (0,))]
        seq += [("o", j, (0,)) for j in (NB - 2, NB - 1)]
        pieces, start = [], {}
        for kind, i, parts in seq:
            start[(kind, i, parts[-1])] = len(pieces)
            start.setdefault((kind, i), len(pieces))
            pieces += [(kind, i, t) for t in groups(parts)]
        n = len(pieces)
        jobs = [[] for _ in range(n + 1)]

        def spread(fn, blk, rows, base, span, tie):
            nc = TM // rows
            for c in range(nc):
                k = base + span[0] + (c * (span[1] - span[0])) // nc + 1
                jobs[min(k, n)].append((fn, blk * TM + c * rows, tie))

        na = TM // AR
        per = len(groups((0, 1, 2))) + (len(groups((0,))) if ILV else 0)
        ASPAN_, LSPAN_, CSPAN_ = [(int(a * per), int(b * per)) for a, b in (ASPAN, LSPAN, CSPAN)]
        A7_, CS_ = [(int(a * len(groups((0,)))), int(b * len(groups((0,))))) for a, b in (A7, CS)]
        g1 = len(groups((0,)))
        for j in range(NB):
            if j + 1 < NB:
                spread(attn_chunk, j, AR, start[("q", j + 1)], ASPAN_, "a" in TIE)
            else:
                spread(attn_chunk, j, AR, start[("o", j - 2)], A7_, "a" in TIE)
            if j == 1:
                spread(ln1_chunk, j, LR, start[("q", 0, 2)] + X1, (0, 0), False)
            elif j == 2:
                spread(ln1_chunk, j, LR, start[("q", 2)] + X2, (0, 0), False)
            elif 2 < j:
                spread(ln1_chunk, j, LR, start[("q", j - 1)], LSPAN_, "l" in TIE)
            if j + 3 < NB:
                spread(ln2_chunk, j, LR, start[("q", j + 3)], CSPAN_, "c" in TIE)
            elif j + 1 < NB:
                spread(ln2_chunk, j, LR, start[("o", j + 1)], CS_, "c" in TIE)
            else:
                spread(ln2_chunk, j, LR, n, (0, 0), False)
        last_c = {}
        for k in range(n + 1):
            for fn, r0, _ in jobs[k]:
                if fn is ln2_chunk:
                    last_c[r0 // TM] = k
        mark = None
        due = [[] for _ in range(n + 1 + DL + DC + DX)]
        stack = contextlib.ExitStack()
        for k in range(n + 1):
            if k % 12 == 0:
                stack.close()
                stack.enter_context(sc("s%d" % k))
            if k == start[("q", 0, 1)] + W1:
                w_copy(1).wait()
                misc[0].start()
                x_cp[2].start()
                prep_w(1)
            if k == start[("q", 0, 2)] + W2:
                w_copy(2).wait()
                for c in misc[1:]:
                    c.start()
                prep_w(2)
            if k == start[("q", 0, 2)] + X1:
                x_cp[1].wait()
            if k == start[("q", 2)] + X2:
                x_cp[2].wait()
                wr_cp.wait()
                misc[0].wait()
                prep_wo()
            for fn, r0, tie in jobs[k]:
                done = fn(r0, mark if tie else None)
                if DL and fn is attn_chunk:
                    due[k + DL].append(done)
                if DX and fn is ln1_chunk:
                    due[min(k + DX, n)].append(done)
                if DC and fn is ln2_chunk and (not CLAST or (r0 + LR) % (TM // CLAST) == 0):
                    due[min(k + DC, n)].append(done)
            for j, kk in last_c.items():
                if kk == k:
                    out_copy(j).start()
            if k < n:
                kind, i, t = pieces[k]
                mark = q_piece(i, t, due[k]) if kind == "q" else o_piece(i, t, due[k])

        stack.close()
        stack.enter_context(sc("tail"))
        bv, bi = best
        gmax = jnp.max(bv, axis=0, keepdims=True)
        cand = jnp.where(bv == gmax, bi + lax.broadcasted_iota(i32, (8, 128), 0), S)
        idx = jnp.min(cand)
        base = pl.multiple_of((idx // 16) * 16, 16)
        h16 = h_v[pl.ds(base, 16), :]
        hn16 = _ln(h16)
        sel = (lax.broadcasted_iota(i32, (16, D), 0) + base) == idx
        xs = jnp.where(sel, hn16, 0.0).astype(bf16)
        for c in misc[1:]:
            c.wait()
        g = jnp.dot(xs, wg_v[...], preferred_element_type=f32)
        u = jnp.dot(xs, wu_v[...], preferred_element_type=f32)
        act = (g * jax.nn.sigmoid(g) * u).astype(bf16)
        y = jnp.dot(act, wd_v[...], preferred_element_type=f32)
        rsel = jnp.sum(hn16 * get_wr(), axis=-1, keepdims=True)
        y = y * jax.nn.sigmoid(rsel)
        fix_v[...] = (h16 + jnp.where(sel, hn16 + y, hn16)).astype(bf16)
        for i in range(NB):
            out_copy(i).wait()
        fix = pltpu.make_async_copy(fix_v, out_hbm.at[pl.ds(base, 16), :], sem_o.at[NB])
        fix.start()
        fix.wait()
        stack.close()

    any_spec = pl.BlockSpec(memory_space=pl.ANY)
    scratch = [
        pltpu.VMEM((D,), bf16),
        pltpu.VMEM((S, D), bf16),
        pltpu.VMEM((D, 3 * D), bf16),
        pltpu.VMEM((D, D), bf16),
        pltpu.VMEM((D, F), bf16),
        pltpu.VMEM((D, F), bf16),
        pltpu.VMEM((F, D), bf16),
        pltpu.VMEM((NT, 960, 128), u32),
        pltpu.VMEM((960, D), u32),
        pltpu.VMEM((NT, 320, 128), u32),
        pltpu.VMEM((320, D), u32),
        pltpu.VMEM((S // 2, D), u32),
        pltpu.VMEM((3 * NT, S + HALO, 128), f32),
        pltpu.VMEM((S // 2, D), u32),
        pltpu.VMEM((S, D), f32),
        pltpu.VMEM((S, D), bf16),
        pltpu.VMEM((16, D), bf16),
        pltpu.SemaphoreType.DMA((4,)),
        pltpu.SemaphoreType.DMA((3 + NT,)),
        pltpu.SemaphoreType.DMA((4,)),
        pltpu.SemaphoreType.DMA((NB + 1,)),
        pltpu.SemaphoreType.REGULAR,
    ]

    def call(A_x, A_wqkv, A_wo, B_x, B_w_r, B_w_gate, B_w_up, B_w_down):
        out = pl.pallas_call(
            kernel,
            out_shape=jax.ShapeDtypeStruct((S, D), bf16),
            in_specs=[any_spec, any_spec, any_spec,
                      any_spec,
                      any_spec, any_spec, any_spec],
            out_specs=any_spec,
            scratch_shapes=scratch,
            compiler_params=pltpu.CompilerParams(vmem_limit_bytes=100 * 1024 * 1024, flags=flags),
        )(A_x.reshape(S, D), A_wqkv, A_wo, B_w_r, B_w_gate, B_w_up, B_w_down)
        return out.reshape(1, S, D)

    return call


_call = make_kernel(TIE='', MM=128, NG=(2,2,1), CLAST=1, DL=8, DC=16, X1=2, CH='a')


@jax.jit
def pallas_sequential_preLN__sliding_local_dilated__moe_arch_mod__prompt_kernel(
    A_x: jax.Array,
    A_wqkv: jax.Array,
    A_wo: jax.Array,
    B_x: jax.Array,
    B_w_r: jax.Array,
    B_w_gate: jax.Array,
    B_w_up: jax.Array,
    B_w_down: jax.Array,
):
    return _call(A_x, A_wqkv, A_wo, B_x, B_w_r, B_w_gate, B_w_up, B_w_down)
```

```python
import math

import jax
import jax.numpy as jnp
from jax import lax
import jax.experimental.pallas as pl
import jax.experimental.pallas.tpu as pltpu

S, D, F = 2048, 640, 1536
H, DH = 32, 20
W, DIL = 8, 2
NT = D // 128
HALO = 16
EPS = 1e-5
QSCALE = (DH ** -0.5) * math.log2(math.e)
TM = 256
MM = 128
NG = (2, 2, 1)
AR = 16
LR = 32
NB = S // TM
ATTN_DUE = 8
LN2_DUE = 16
f32, bf16, u32, i32 = jnp.float32, jnp.bfloat16, jnp.uint32, jnp.int32


def _pack(v):
    return pltpu.bitcast(v.astype(bf16), u32)


def _unpack(v):
    return pltpu.bitcast(v, bf16)


def _tiles(v):
    return [v[:, t * 128:(t + 1) * 128] for t in range(NT)]


def _rowsum(ts):
    acc = ts[0]
    for t in ts[1:]:
        acc = acc + t
    return jnp.sum(acc, axis=-1, keepdims=True)


def _groups(parts):
    out = []
    for m in range(TM // MM):
        for p in parts:
            t0 = p * NT
            for g in NG:
                out.append((m, t0, g))
                t0 += g
    return out


def _kernel(x_hbm, wqkv_hbm, wo_hbm, wr_hbm, wg_hbm, wu_hbm, wd_hbm, out_hbm,
            wr_v, x_v, wqkv_v, wo_v, wg_v, wu_v, wd_v,
            wt_u, wp, wo_u, wop,
            xn, qkv, o_v, h_v, out_v, fix_v, st_v,
            sem_x, sem_w, sem_m, sem_o, sem_r):

    xcuts = [0, TM, 2 * TM, S]
    x_cp = [pltpu.make_async_copy(x_hbm.at[pl.ds(a, b - a), :], x_v.at[pl.ds(a, b - a), :], sem_x.at[k])
            for k, (a, b) in enumerate(zip(xcuts[:-1], xcuts[1:]))]
    w_cp = [pltpu.make_async_copy(wqkv_hbm.at[:, pl.ds(p * D, D)], wqkv_v.at[:, pl.ds(p * D, D)], sem_w.at[p])
            for p in range(3)]
    wo_cp = pltpu.make_async_copy(wo_hbm, wo_v, sem_m.at[0])
    ffn_cp = [pltpu.make_async_copy(wg_hbm, wg_v, sem_m.at[1]),
              pltpu.make_async_copy(wu_hbm, wu_v, sem_m.at[2]),
              pltpu.make_async_copy(wd_hbm, wd_v, sem_m.at[3])]
    wr_cp = pltpu.make_async_copy(wr_hbm, wr_v, sem_x.at[3])
    out_cp = [pltpu.make_async_copy(out_v.at[pl.ds(i * TM, TM), :], out_hbm.at[pl.ds(i * TM, TM), :], sem_o.at[i])
              for i in range(NB)]

    x_cp[0].start()
    w_cp[0].start()

    never = pl.semaphore_read(sem_r) > 0
    chain = []

    def after(lhs, deps):
        if not deps:
            return lhs
        d = deps[0]
        for e in deps[1:]:
            d = d | e
        head = jnp.where(never, d, lhs[0:8, 0:128])
        top = jnp.concatenate([head, lhs[0:8, 128:]], axis=1)
        return jnp.concatenate([top, lhs[8:]], axis=0)

    def prep_w(p):
        for kt in range(NT):
            wt = wqkv_v[pl.ds(kt * 128, 128), pl.ds(p * D, D)].T
            wt_u[kt, pl.ds(p * 320, 320), :] = pltpu.bitcast(wt, u32)
        for kt in range(NT):
            for j in range(NT):
                for a in range(2):
                    wp[pl.ds(p * 320 + j * 64 + a * 32, 32), pl.ds(kt * 128, 128)] = (
                        wt_u[kt, pl.ds(p * 320 + 2 * j + a, 32, stride=10), :])

    def prep_wo():
        for nt in range(NT):
            wo_u[nt] = pltpu.bitcast(wo_v[:, pl.ds(nt * 128, 128)], u32)
        for nt in range(NT):
            for j in range(NT):
                for a in range(2):
                    wop[pl.ds(j * 64 + a * 32, 32), pl.ds(nt * 128, 128)] = (
                        wo_u[nt, pl.ds(2 * j + a, 32, stride=10), :])

    def ln1_chunk(r0):
        x = x_v[pl.ds(r0, LR), :].astype(f32)
        c = x - _rowsum(_tiles(x)) * (1.0 / D)
        var = _rowsum(_tiles(c * c)) * (1.0 / D)
        xn[pl.ds(r0 // 2, LR // 2), :] = _pack(c * lax.rsqrt(var + EPS))

    def q_piece(i, t, deps):
        m, t0, nt = t
        r0 = i * TM + m * MM
        lhs = _unpack(after(xn[pl.ds(r0 // 2, MM // 2), :], deps))
        res = lax.dot_general(lhs, _unpack(wp[pl.ds(t0 * 64, nt * 64), :]),
                              (((1,), (1,)), ((), ())), preferred_element_type=f32)
        for u in range(nt):
            qkv[t0 + u, pl.ds(HALO + r0, MM), :] = res[:, u * 128:(u + 1) * 128]

    def o_piece(i, t, deps):
        m, t0, nt = t
        r0 = i * TM + m * MM
        cols = pl.ds(t0 * 128, nt * 128)
        res = jnp.dot(_unpack(after(o_v[pl.ds(r0 // 2, MM // 2), :], deps)),
                      _unpack(wop[:, cols]), preferred_element_type=f32)
        h_v[pl.ds(r0, MM), cols] = res + x_v[pl.ds(r0, MM), cols].astype(f32)

    swap = lax.broadcasted_iota(i32, (AR, 128), 1) ^ 1

    def attn_chunk(r0):
        sc = jnp.full((8, 128), QSCALE, f32)
        if chain:
            sc = jnp.where(never, chain[-1], sc)
        sc = jnp.concatenate([sc] * (AR // 8), axis=0)
        q = [qkv[t, pl.ds(HALO + r0, AR), :] * sc for t in range(NT)]
        accs = []
        for w in range(W):
            acc = None
            for t in range(NT):
                e = q[t] * qkv[NT + t, pl.ds(HALO + r0 - DIL * w, AR), :]
                acc = e if acc is None else acc + e
            accs.append(acc)
        rolled = [pltpu.roll(a, 64, 1) for a in accs]
        accs = [a + r for a, r in zip(accs, rolled)]
        chain.append(accs[-1][0:8])
        swapped = [jnp.take_along_axis(a, swap, axis=1) for a in accs]
        logits = []
        for w in range(W):
            acc = accs[w] + swapped[w]
            if r0 < DIL * w:
                row = r0 + lax.broadcasted_iota(i32, (AR, 128), 0)
                acc = jnp.where(row >= DIL * w, acc, -1e9)
            logits.append(acc)
        m = logits[0]
        for w in range(1, W):
            m = jnp.maximum(m, logits[w])
        es = [jnp.exp2(l - m) for l in logits]
        ssum = es[0]
        for w in range(1, W):
            ssum = ssum + es[w]
        inv = 1.0 / ssum
        done = None
        for t in range(NT):
            acc = None
            for w in range(W):
                e = es[w] * qkv[2 * NT + t, pl.ds(HALO + r0 - DIL * w, AR), :]
                acc = e if acc is None else acc + e
            packed = _pack(acc * inv)
            o_v[pl.ds(r0 // 2, AR // 2), pl.ds(t * 128, 128)] = packed
            done = packed if done is None else done | packed
        return done

    best = [jnp.full((8, 128), -jnp.inf, f32), jnp.zeros((8, 128), i32)]
    wr_box = []

    def ln2_chunk(r0):
        if not wr_box:
            wr_box.append(wr_v[...].astype(f32).reshape(1, D))
        h = h_v[pl.ds(r0, LR), :]
        m = _rowsum(_tiles(h)) * (1.0 / D)
        c = h - m
        var = _rowsum(_tiles(c * c)) * (1.0 / D)
        cw = _rowsum(_tiles(c * wr_box[0]))
        rstd = lax.rsqrt(var + EPS)
        st_v[0, pl.ds(r0, LR), :] = jnp.broadcast_to(m, (LR, 128))
        st_v[1, pl.ds(r0, LR), :] = jnp.broadcast_to(rstd, (LR, 128))
        out_v[pl.ds(r0, LR), :] = (h + c * rstd).astype(bf16)
        r = jnp.broadcast_to(cw * rstd, (LR, 128))
        bv, bi = best
        for g in range(LR // 8):
            rg = r[g * 8:(g + 1) * 8]
            upd = rg > bv
            bv = jnp.where(upd, rg, bv)
            bi = jnp.where(upd, r0 + g * 8, bi)
        best[0], best[1] = bv, bi
        return pltpu.bitcast(bv, u32)

    zero_halo = jnp.zeros((HALO, 128), f32)
    for t in range(NT, 3 * NT):
        qkv[t, pl.ds(0, HALO), :] = zero_halo

    x_cp[0].wait()
    w_cp[1].start()
    wr_cp.start()
    for r0 in range(0, TM, LR):
        ln1_chunk(r0)
    w_cp[0].wait()
    w_cp[2].start()
    x_cp[1].start()
    prep_w(0)

    seq = [("q", 0, (p,)) for p in range(3)] + [("q", 1, (0, 1, 2))]
    for i in range(2, NB):
        seq += [("q", i, (0, 1, 2)), ("o", i - 2, (0,))]
    seq += [("o", j, (0,)) for j in (NB - 2, NB - 1)]
    pieces, start = [], {}
    for kind, i, parts in seq:
        start[(kind, i, parts[-1])] = len(pieces)
        start.setdefault((kind, i), len(pieces))
        pieces += [(kind, i, t) for t in _groups(parts)]
    n = len(pieces)
    jobs = [[] for _ in range(n + 1)]

    def spread(fn, blk, rows, base, lo, hi):
        nc = TM // rows
        for c in range(nc):
            k = base + lo + (c * (hi - lo)) // nc + 1
            jobs[min(k, n)].append((fn, blk * TM + c * rows))

    nq, no = len(_groups((0, 1, 2))), len(_groups((0,)))
    x1_at = start[("q", 0, 2)] + 2
    x2_at = start[("q", 2)] - 4
    for j in range(NB):
        if j + 1 < NB:
            spread(attn_chunk, j, AR, start[("q", j + 1)], 0, nq)
        else:
            spread(attn_chunk, j, AR, start[("o", j - 2)], 0, 2 * no)
        if j == 1:
            spread(ln1_chunk, j, LR, x1_at, 0, 0)
        elif j == 2:
            spread(ln1_chunk, j, LR, x2_at, 0, 0)
        elif j > 2:
            spread(ln1_chunk, j, LR, start[("q", j - 1)], 0, int(0.67 * nq))
        if j + 3 < NB:
            spread(ln2_chunk, j, LR, start[("q", j + 3)], 0, nq)
        elif j + 1 < NB:
            spread(ln2_chunk, j, LR, start[("o", j + 1)], 0, no)
        else:
            spread(ln2_chunk, j, LR, n, 0, 0)

    due = [[] for _ in range(n + 1 + ATTN_DUE)]
    for k in range(n + 1):
        if k == start[("q", 0, 1)] - 3:
            w_cp[1].wait()
            wo_cp.start()
            x_cp[2].start()
            prep_w(1)
        if k == start[("q", 0, 2)] - 3:
            w_cp[2].wait()
            for c in ffn_cp:
                c.start()
            prep_w(2)
        if k == x1_at:
            x_cp[1].wait()
        if k == x2_at:
            x_cp[2].wait()
            wr_cp.wait()
            wo_cp.wait()
            prep_wo()
        for fn, r0 in jobs[k]:
            done = fn(r0)
            if fn is attn_chunk:
                due[k + ATTN_DUE].append(done)
            if fn is ln2_chunk and (r0 + LR) % TM == 0:
                due[min(k + LN2_DUE, n)].append(done)
                out_cp[r0 // TM].start()
        if k < n:
            kind, i, t = pieces[k]
            (q_piece if kind == "q" else o_piece)(i, t, due[k])

    bv, bi = best
    gmax = jnp.max(bv, axis=0, keepdims=True)
    cand = jnp.where(bv == gmax, bi + lax.broadcasted_iota(i32, (8, 128), 0), S)
    idx = jnp.min(cand)
    base = pl.multiple_of((idx // 16) * 16, 16)
    h16 = h_v[pl.ds(base, 16), :]
    hn16 = (h16 - st_v[0, pl.ds(base, 16), 0:1]) * st_v[1, pl.ds(base, 16), 0:1]
    sel = (lax.broadcasted_iota(i32, (16, D), 0) + base) == idx
    xs = jnp.where(sel, hn16, 0.0).astype(bf16)
    for c in ffn_cp:
        c.wait()
    g = jnp.dot(xs, wg_v[...], preferred_element_type=f32)
    u = jnp.dot(xs, wu_v[...], preferred_element_type=f32)
    act = (g * jax.nn.sigmoid(g) * u).astype(bf16)
    y = jnp.dot(act, wd_v[...], preferred_element_type=f32)
    y = y * jax.nn.sigmoid(gmax[:, 0:1])
    fix_v[...] = (h16 + jnp.where(sel, hn16 + y, hn16)).astype(bf16)
    for c in out_cp:
        c.wait()
    fix = pltpu.make_async_copy(fix_v, out_hbm.at[pl.ds(base, 16), :], sem_o.at[NB])
    fix.start()
    fix.wait()


@jax.jit
def pallas_sequential_preLN__sliding_local_dilated__moe_arch_mod__prompt_kernel(
    A_x: jax.Array,
    A_wqkv: jax.Array,
    A_wo: jax.Array,
    B_x: jax.Array,
    B_w_r: jax.Array,
    B_w_gate: jax.Array,
    B_w_up: jax.Array,
    B_w_down: jax.Array,
):
    del B_x
    any_spec = pl.BlockSpec(memory_space=pl.ANY)
    scratch = [
        pltpu.VMEM((D,), bf16),
        pltpu.VMEM((S, D), bf16),
        pltpu.VMEM((D, 3 * D), bf16),
        pltpu.VMEM((D, D), bf16),
        pltpu.VMEM((D, F), bf16),
        pltpu.VMEM((D, F), bf16),
        pltpu.VMEM((F, D), bf16),
        pltpu.VMEM((NT, 960, 128), u32),
        pltpu.VMEM((960, D), u32),
        pltpu.VMEM((NT, 320, 128), u32),
        pltpu.VMEM((320, D), u32),
        pltpu.VMEM((S // 2, D), u32),
        pltpu.VMEM((3 * NT, S + HALO, 128), f32),
        pltpu.VMEM((S // 2, D), u32),
        pltpu.VMEM((S, D), f32),
        pltpu.VMEM((S, D), bf16),
        pltpu.VMEM((16, D), bf16),
        pltpu.VMEM((2, S, 128), f32),
        pltpu.SemaphoreType.DMA((4,)),
        pltpu.SemaphoreType.DMA((3,)),
        pltpu.SemaphoreType.DMA((4,)),
        pltpu.SemaphoreType.DMA((NB + 1,)),
        pltpu.SemaphoreType.REGULAR,
    ]
    out = pl.pallas_call(
        _kernel,
        out_shape=jax.ShapeDtypeStruct((S, D), bf16),
        in_specs=[any_spec] * 7,
        out_specs=any_spec,
        scratch_shapes=scratch,
        compiler_params=pltpu.CompilerParams(vmem_limit_bytes=100 * 1024 * 1024),
    )(A_x.reshape(S, D), A_wqkv, A_wo, B_w_r, B_w_gate, B_w_up, B_w_down)
    return out.reshape(1, S, D)
```
